```python
import os as _os
_os.environ.setdefault("JAX_PLATFORMS", "cpu")
import jax
import jax.numpy as jnp

def _softmax(x, axis=-1):
    return jax.nn.softmax(x, axis=axis)
def _gelu(x):
    return jax.nn.gelu(x, approximate=True)
def _silu(x):
    return jax.nn.silu(x)
def _sigmoid(x):
    return jax.nn.sigmoid(x)
def _layernorm(x, axis=-1, eps=1e-5):
    m = jnp.mean(x, axis=axis, keepdims=True)
    v = jnp.var(x, axis=axis, keepdims=True)
    return (x - m) / jnp.sqrt(v + eps)
def _scatter_add(tgt, idx, src, axis=0):
    return tgt.at[idx].add(src)
def _segment_sum(src, seg, n):
    return jax.ops.segment_sum(src, seg, n)
class _Rng:
    def __init__(self, key):
        self._k = key
    def _next(self):
        self._k, sub = jax.random.split(self._k)
        return sub
    def normal(self, shape):
        return jax.random.normal(self._next(), shape, dtype=jnp.bfloat16)
    def randint(self, lo, hi, shape):
        return jax.random.randint(self._next(), shape, lo, hi, dtype=jnp.int32)
    def uniform(self, shape, lo=0.0, hi=1.0):
        return jax.random.uniform(self._next(), shape, jnp.bfloat16, lo, hi)
    def permutation(self, n):
        return jax.random.permutation(self._next(), n)


kernel_name = 'sequential_preLN__mha_block__moe_arch_mod__prompt'

def setup_inputs():
    _rng = _Rng(jax.random.key(int.from_bytes(__import__("os").urandom(4), "little")))
    _w = (lambda a: (lambda t: t.astype(jnp.bfloat16) if jnp.issubdtype(t.dtype, jnp.floating) else t)(jnp.asarray(a)))
    def _A_setup():
        B, S, D, H = 1, 2048, 640, 32
        return {
            "x": _w((lambda *s: _rng.normal(s) * 0.05)(B, S, D)),
            "wqkv": _w((lambda *s: _rng.normal(s) * 0.05)(D, 3 * D)),
            "wo": _w((lambda *s: _rng.normal(s) * 0.05)(D, D)),
        }
    _A_in = _A_setup()

    def _B_setup():
        B, S, D, F, C = 1, 2048, 640, 1536, 1
        return {
            "x": _w((lambda *s: _rng.normal(s) * 0.05)(B, S, D)),
            "w_r": _w((lambda *s: _rng.normal(s) * 0.05)(D)),
            "w_gate": _w((lambda *s: _rng.normal(s) * 0.05)(D, F)),
            "w_up": _w((lambda *s: _rng.normal(s) * 0.05)(D, F)),
            "w_down": _w((lambda *s: _rng.normal(s) * 0.05)(F, D)),
        }
    _B_in = _B_setup()

    return {
        "A_x": _A_in["x"],
        "A_wqkv": _A_in["wqkv"],
        "A_wo": _A_in["wo"],
        "B_x": _B_in["x"],
        "B_w_r": _B_in["w_r"],
        "B_w_gate": _B_in["w_gate"],
        "B_w_up": _B_in["w_up"],
        "B_w_down": _B_in["w_down"],
    }

def reference(A_x, A_wqkv, A_wo, B_x, B_w_r, B_w_gate, B_w_up, B_w_down):
    def _A_ref(x, wqkv, wo):
        B, S, D = x.shape
        H = 32
        Dh = D // H
        qkv = (lambda x, *d: x.transpose(*d))((x @ wqkv).reshape(B, S, 3, H, Dh), 2, 0, 3, 1, 4)
        q, k, v = qkv[0], qkv[1], qkv[2]
        scores = jnp.einsum("bhqd,bhkd->bhqk", q, k) * (Dh ** -0.5)
        p = _softmax(scores, axis=-1)
        o = jnp.einsum("bhqk,bhkd->bhqd", p, v)
        return (lambda x, *d: x.transpose(*d))(o, 0, 2, 1, 3).reshape(B, S, D) @ wo

    def _B_ref(x, w_r, w_gate, w_up, w_down):
        B, S, D = x.shape
        C = 1
        r = x @ w_r
        idx = jnp.argsort(-r, axis=-1)[:, :C]
        idx_e = jnp.repeat(idx.reshape(B, C, 1), D, axis=2)
        x_sel = jnp.take_along_axis(x, idx_e, axis=1)
        g = _silu(x_sel @ w_gate)
        u = x_sel @ w_up
        y = (g * u) @ w_down
        r_sel = _sigmoid(jnp.take_along_axis(r, idx, axis=1))
        y = y * r_sel.reshape(B, C, 1)
        b_off = (jnp.arange(B) * S).reshape(B, 1)
        flat_idx = (idx + b_off).reshape(B * C)
        zero = (x * 0.0).reshape(B * S, D)
        upd = _scatter_add(zero, flat_idx, y.reshape(B * C, D), axis=0)
        return x + upd.reshape(B, S, D)

    x = A_x
    h = x + _A_ref(_layernorm(x, axis=-1), A_wqkv, A_wo)
    h2 = h + _B_ref(_layernorm(h, axis=-1), B_w_r, B_w_gate, B_w_up, B_w_down)
    return h2
```

```python
import functools

import jax
import jax.numpy as jnp
import jax.experimental.pallas as pl
import jax.experimental.pallas.tpu as pltpu

H = 32
DH = 20
HP = 32
G = 8
EPS = 1e-5


def _ln(x):
    m = jnp.mean(x, axis=-1, keepdims=True)
    c = x - m
    v = jnp.mean(c * c, axis=-1, keepdims=True)
    return c * jax.lax.rsqrt(v + EPS)


def _kernel(x_ref, wqkv_ref, wo_ref, wr_ref, wg_ref, wu_ref, wd_ref, o_ref,
            q_sc, k_sc, v_sc, ln2_sc, sum_sc, r_sc, *, S, D, tp, tq):
    DP = H * HP
    lane = jax.lax.broadcasted_iota(jnp.int32, (1, DP), 1)
    is_pad = (lane % HP) >= DH

    def proj(i, _):
        r0 = pl.multiple_of(i * tp, tp)
        xb = x_ref[pl.ds(r0, tp), :].astype(jnp.float32)
        ln1 = _ln(xb).astype(jnp.bfloat16)
        q = jnp.dot(ln1, wqkv_ref[:, 0:DP], preferred_element_type=jnp.float32)
        q_sc[pl.ds(r0, tp), :] = (q * (DH ** -0.5)).astype(jnp.bfloat16)
        k = jnp.dot(ln1, wqkv_ref[:, DP:2 * DP], preferred_element_type=jnp.float32)
        k_sc[pl.ds(r0, tp), :] = k.astype(jnp.bfloat16)
        v = jnp.dot(ln1, wqkv_ref[:, 2 * DP:3 * DP], preferred_element_type=jnp.float32)
        v_sc[pl.ds(r0, tp), :] = jnp.where(is_pad, 1.0, v).astype(jnp.bfloat16)
        return 0

    jax.lax.fori_loop(0, S // tp, proj, 0)

    lane128 = jax.lax.broadcasted_iota(jnp.int32, (1, 128), 1)

    def attn(i, _):
        r0 = pl.multiple_of(i * tq, tq)
        outs = []
        for g in range(G):
            qg = q_sc[pl.ds(r0, tq), g * 128:(g + 1) * 128].astype(jnp.float32)
            kg = k_sc[:, g * 128:(g + 1) * 128]
            vg = v_sc[:, g * 128:(g + 1) * 128]
            og = jnp.zeros((tq, 128), jnp.float32)
            for j in range(128 // HP):
                mask = (lane128 >= j * HP) & (lane128 < j * HP + DH)
                qm = jnp.where(mask, qg, 0.0).astype(jnp.bfloat16)
                s = jax.lax.dot_general(qm, kg, (((1,), (1,)), ((), ())),
                                        preferred_element_type=jnp.float32)
                m = jnp.max(s, axis=1, keepdims=True)
                p = jnp.exp(s - m).astype(jnp.bfloat16)
                res = jnp.dot(p, vg, preferred_element_type=jnp.float32)
                l = res[:, j * HP + DH:j * HP + DH + 1]
                og = og + jnp.where(mask, res / l, 0.0)
            outs.append(og.astype(jnp.bfloat16))
        o = jnp.concatenate(outs, axis=1)
        a = jnp.dot(o, wo_ref[...], preferred_element_type=jnp.float32)
        h = x_ref[pl.ds(r0, tq), :].astype(jnp.float32) + a
        ln2 = _ln(h)
        ln2_sc[pl.ds(r0, tq), :] = ln2
        sum_sc[pl.ds(r0, tq), :] = h + ln2
        o_ref[pl.ds(r0, tq), :] = (h + ln2).astype(o_ref.dtype)
        r_sc[pl.ds(r0, tq), :] = jnp.sum(ln2 * wr_ref[...].astype(jnp.float32),
                                         axis=1, keepdims=True)
        return 0

    jax.lax.fori_loop(0, S // tq, attn, 0)

    r = r_sc[...]
    rmax = jnp.max(r)
    rows = jax.lax.broadcasted_iota(jnp.int32, (S, 1), 0)
    idx = jnp.min(jnp.where(r == rmax, rows, S))
    xs = jnp.broadcast_to(ln2_sc[pl.ds(idx, 1), :], (8, D)).astype(jnp.bfloat16)
    gt = jnp.dot(xs, wg_ref[...], preferred_element_type=jnp.float32)
    u = jnp.dot(xs, wu_ref[...], preferred_element_type=jnp.float32)
    act = (gt * jax.nn.sigmoid(gt) * u).astype(jnp.bfloat16)
    y = jnp.dot(act, wd_ref[...], preferred_element_type=jnp.float32)[0:1, :]
    y = y * jax.nn.sigmoid(rmax)
    base = pl.multiple_of((idx // 16) * 16, 16)
    rr = base + jax.lax.broadcasted_iota(jnp.int32, (16, 1), 0)
    blk = sum_sc[pl.ds(base, 16), :] + jnp.where(rr == idx, y, 0.0)
    o_ref[pl.ds(base, 16), :] = blk.astype(o_ref.dtype)


@jax.jit
def pallas_sequential_preLN__mha_block__moe_arch_mod__prompt_kernel(
    A_x: jax.Array,
    A_wqkv: jax.Array,
    A_wo: jax.Array,
    B_x: jax.Array,
    B_w_r: jax.Array,
    B_w_gate: jax.Array,
    B_w_up: jax.Array,
    B_w_down: jax.Array,
):
    B, S, D = A_x.shape
    assert B == 1 and D == H * DH
    x = A_x.reshape(S, D)
    wqkv = jnp.pad(A_wqkv.reshape(D, 3 * H, DH), ((0, 0), (0, 0), (0, HP - DH)))
    wqkv = wqkv.reshape(D, 3 * H * HP)
    wo = jnp.pad(A_wo.reshape(H, DH, D), ((0, 0), (0, HP - DH), (0, 0)))
    wo = wo.reshape(H * HP, D)
    wr = B_w_r.reshape(1, D)
    DP = H * HP
    out = pl.pallas_call(
        functools.partial(_kernel, S=S, D=D, tp=512, tq=512),
        out_shape=jax.ShapeDtypeStruct((S, D), A_x.dtype),
        scratch_shapes=[
            pltpu.VMEM((S, DP), jnp.bfloat16),
            pltpu.VMEM((S, DP), jnp.bfloat16),
            pltpu.VMEM((S, DP), jnp.bfloat16),
            pltpu.VMEM((S, D), jnp.float32),
            pltpu.VMEM((S, D), jnp.float32),
            pltpu.VMEM((S, 1), jnp.float32),
        ],
        compiler_params=pltpu.CompilerParams(vmem_limit_bytes=100 << 20),
    )(x, wqkv, wo, wr, B_w_gate, B_w_up, B_w_down)
    return out.reshape(B, S, D)
```
